```python
import os as _os
_os.environ.setdefault("JAX_PLATFORMS", "cpu")
import jax
import jax.numpy as jnp

def _softmax(x, axis=-1):
    return jax.nn.softmax(x, axis=axis)
def _gelu(x):
    return jax.nn.gelu(x, approximate=True)
def _silu(x):
    return jax.nn.silu(x)
def _sigmoid(x):
    return jax.nn.sigmoid(x)
def _layernorm(x, axis=-1, eps=1e-5):
    m = jnp.mean(x, axis=axis, keepdims=True)
    v = jnp.var(x, axis=axis, keepdims=True)
    return (x - m) / jnp.sqrt(v + eps)
def _scatter_add(tgt, idx, src, axis=0):
    return tgt.at[idx].add(src)
def _segment_sum(src, seg, n):
    return jax.ops.segment_sum(src, seg, n)
class _Rng:
    def __init__(self, key):
        self._k = key
    def _next(self):
        self._k, sub = jax.random.split(self._k)
        return sub
    def normal(self, shape):
        return jax.random.normal(self._next(), shape, dtype=jnp.bfloat16)
    def randint(self, lo, hi, shape):
        return jax.random.randint(self._next(), shape, lo, hi, dtype=jnp.int32)
    def uniform(self, shape, lo=0.0, hi=1.0):
        return jax.random.uniform(self._next(), shape, jnp.bfloat16, lo, hi)
    def permutation(self, n):
        return jax.random.permutation(self._next(), n)


kernel_name = 'parallel_sum__ssm_conv_s5__glu_gated_swiglu__prompt'

def setup_inputs():
    _rng = _Rng(jax.random.key(int.from_bytes(__import__("os").urandom(4), "little")))
    _w = (lambda a: (lambda t: t.astype(jnp.bfloat16) if jnp.issubdtype(t.dtype, jnp.floating) else t)(jnp.asarray(a)))
    def _A_setup():
        B, S, D = 1, 2048, 640
        P = D
        Lambda_re = -0.5 * jnp.exp((lambda *s: _rng.normal(s) * 0.4)(P))
        Lambda_im = (lambda *s: _rng.normal(s) * 0.4)(P) * 1.0
        B_re = (lambda *s: _rng.normal(s) * 0.4)(P, D) * (D ** -0.5)
        B_im = (lambda *s: _rng.normal(s) * 0.4)(P, D) * (D ** -0.5)
        C_re = (lambda *s: _rng.normal(s) * 0.4)(D, P) * (P ** -0.5)
        C_im = (lambda *s: _rng.normal(s) * 0.4)(D, P) * (P ** -0.5)
        log_dt = (lambda *s: _rng.normal(s) * 0.4)(P) * 0.3 - 2.0
        Dskip = (lambda *s: _rng.normal(s) * 0.4)(D)
        return {
            "x": _w((lambda *s: _rng.normal(s) * 0.05)(B, S, D)),
            "Lambda_re": _w(Lambda_re),
            "Lambda_im": _w(Lambda_im),
            "B_re": _w(B_re),
            "B_im": _w(B_im),
            "C_re": _w(C_re),
            "C_im": _w(C_im),
            "log_dt": _w(log_dt),
            "Dskip": _w(Dskip),
        }
    _A_in = _A_setup()

    def _B_setup():
        B, S, D, F = 1, 2048, 640, 1728
        return {
            "x": _w((lambda *s: _rng.normal(s) * 0.05)(B, S, D)),
            "w1": _w((lambda *s: _rng.normal(s) * 0.1)(D, F) * (2.0 / D) ** 0.5),
            "w3": _w((lambda *s: _rng.normal(s) * 0.1)(D, F) * (2.0 / D) ** 0.5),
            "w2": _w((lambda *s: _rng.normal(s) * 0.1)(F, D) * (2.0 / F) ** 0.5),
        }
    _B_in = _B_setup()

    return {
        "A_x": _A_in["x"],
        "A_Lambda_re": _A_in["Lambda_re"],
        "A_Lambda_im": _A_in["Lambda_im"],
        "A_B_re": _A_in["B_re"],
        "A_B_im": _A_in["B_im"],
        "A_C_re": _A_in["C_re"],
        "A_C_im": _A_in["C_im"],
        "A_log_dt": _A_in["log_dt"],
        "A_Dskip": _A_in["Dskip"],
        "B_x": _B_in["x"],
        "B_w1": _B_in["w1"],
        "B_w3": _B_in["w3"],
        "B_w2": _B_in["w2"],
    }

def reference(A_x, A_Lambda_re, A_Lambda_im, A_B_re, A_B_im, A_C_re, A_C_im, A_log_dt, A_Dskip, B_x, B_w1, B_w3, B_w2):
    def _A_ref(x, Lambda_re, Lambda_im, B_re, B_im, C_re, C_im, log_dt, Dskip):
        Bsz, L, H = x.shape
        Lam = Lambda_re + 1j * Lambda_im
        Bmat = B_re + 1j * B_im
        Cmat = C_re + 1j * C_im
        dt = jnp.exp(log_dt)
        Lam_bar = jnp.exp(dt * Lam)
        B_bar = ((Lam_bar - 1.0) / Lam)[:, None] * Bmat
        Bu = jnp.einsum("bld,pd->blp", x + 0j, B_bar)
        h = jnp.zeros_like(Bu[:, 0, :])
        hs = []
        for t in range(L):
            h = Lam_bar[None, :] * h + Bu[:, t, :]
            hs.append(h)
        hseq = jnp.stack(hs, 1)
        y = 2.0 * jnp.einsum("blp,dp->bld", hseq, Cmat).real + x * Dskip[None, None, :]
        return y

    def _B_ref(x, w1, w3, w2):
        gate = jnp.einsum("bsd,df->bsf", x, w1)
        up = jnp.einsum("bsd,df->bsf", x, w3)
        h = _silu(gate) * up
        out = jnp.einsum("bsf,fd->bsd", h, w2)
        return out

    x = A_x
    xn = _layernorm(x, axis=-1)
    return x + _A_ref(xn, A_Lambda_re, A_Lambda_im, A_B_re, A_B_im, A_C_re, A_C_im, A_log_dt, A_Dskip) + _B_ref(xn, B_w1, B_w3, B_w2)
```

```python
import functools
import jax
import jax.numpy as jnp
from jax import lax
import jax.experimental.pallas as pl
import jax.experimental.pallas.tpu as pltpu

L, D, P, F = 2048, 640, 640, 1728
NC = D // 128
FM = (F // 128) * 128
FT = F - FM
NFT = FM // 128
EPS = 1e-5

NT_DIMS = (((1,), (1,)), ((), ()))
NN_DIMS = (((1,), (0,)), ((), ()))

T_CR, T_CI, T_NCR, T_DSK = 0, 1, 2, 3
T_A = 4
T_T = 6
N_TAB = 12


def _bf(x):
    return x.astype(jnp.bfloat16).astype(jnp.float32)


def _cmac(xr, xi, ar, ai, yr, yi):
    return xr + ar * yr - ai * yi, xi + ar * yi + ai * yr


def _dot(a, b, dims):
    return lax.dot_general(a, b, dims, preferred_element_type=jnp.float32)


def make_kernel(TL=256, GU_CHUNK=2, extra=0, bseg=(2, 6), wgroups=(1, 5), stagger=0, once=False):
    NS = L // TL
    G = TL // 64

    gu_chunks = []
    t = 0
    while t < NFT:
        n = min(GU_CHUNK, NFT - t)
        gu_chunks.append((t, n))
        t += n
    NGU = len(gu_chunks)
    wb = [0] + list(wgroups) + [NGU + 1]
    NWG = len(wb) - 1
    def wgroup_of(ci):
        for k in range(NWG):
            if wb[k] <= ci < wb[k + 1]:
                return k
    bb = [0] + list(bseg) + [2 * NC]
    NBS = len(bb) - 1

    S_X0 = 0
    S_B = 1
    S_W = S_B + NBS - 1
    S_XR = S_W + NWG
    N_SEM = S_XR + 1

    def kernel(x_hbm, lre_hbm, lim_hbm, bre_hbm, bim_hbm, cre_hbm, cim_hbm, ldt_hbm, dsk_hbm,
               w1t_hbm, w3t_hbm, w2_hbm, o_hbm,
               xs, pv0, pv1, pv2, pv3, bcat, w13, ccat, w2v, tab, hst, xn_s, base_s, yp_s, h_s, act_s, obuf, bu_s,
               sem, sem_o):
        pv = (pv0, pv1, pv2, pv3)

        def x_copies(blk):
            s = S_X0 if blk == 0 else (S_B if blk == 1 else S_XR)
            return [pltpu.make_async_copy(
                x_hbm.at[0, pl.ds(blk * TL, TL), pl.ds(c * 128, 128)],
                xs.at[blk, c], sem.at[s]) for c in range(NC)]

        def p_copies():
            return [pltpu.make_async_copy(src, pv[k], sem.at[S_X0])
                    for k, src in enumerate((lre_hbm, lim_hbm, ldt_hbm, dsk_hbm))]

        def b_copies(k):
            r0, r1 = bb[k] * 128, bb[k + 1] * 128
            s = sem.at[S_B + k]
            cps = []
            for src, o in ((bre_hbm, 0), (bim_hbm, P)):
                a, b = max(r0, o), min(r1, o + P)
                if a < b:
                    cps.append(pltpu.make_async_copy(src.at[pl.ds(a - o, b - a), :],
                                                     bcat.at[pl.ds(a, b - a), :], s))
            return cps

        def w13_copies(ci):
            if ci == NGU:
                r, s0, d0 = FT, FM, 2 * FM
            else:
                t0, n = gu_chunks[ci]
                r, s0, d0 = n * 128, t0 * 128, 2 * t0 * 128
            s = sem.at[S_W + wgroup_of(ci)]
            return [pltpu.make_async_copy(w1t_hbm.at[pl.ds(s0, r), :], w13.at[pl.ds(d0, r), :], s),
                    pltpu.make_async_copy(w3t_hbm.at[pl.ds(s0, r), :], w13.at[pl.ds(d0 + r, r), :], s)]

        def c_copies():
            s = sem.at[S_W + NWG - 1]
            return [pltpu.make_async_copy(cre_hbm, ccat.at[:, pl.ds(0, P)], s),
                    pltpu.make_async_copy(cim_hbm, ccat.at[:, pl.ds(P, P)], s)]

        def w2_copies():
            return [pltpu.make_async_copy(w2_hbm, w2v, sem.at[S_W + NWG - 1])]

        def group_copies(k):
            cps = []
            if k == 0:
                cps += b_copies(NBS - 1)
            for ci in range(wb[k], wb[k + 1]):
                cps += w13_copies(ci)
            if k == NWG - 1:
                cps += w2_copies() + c_copies()
            return cps

        def o_copy(slot, blk, c):
            return pltpu.make_async_copy(
                obuf.at[slot, c], o_hbm.at[0, pl.ds(blk * TL, TL), pl.ds(c * 128, 128)],
                sem_o.at[slot])

        def start(cps):
            for cp in cps:
                cp.start()

        def wait(cps):
            for cp in cps:
                cp.wait()

        x32 = xs.bitcast(jnp.uint32)

        def ld16(ref, r0, nr, cols=slice(None)):
            return pltpu.bitcast(ref[pl.ds(r0 // 2, nr // 2), cols], jnp.bfloat16)

        def st16(ref, r0, cols, val):
            ref[pl.ds(r0 // 2, val.shape[0] // 2), cols] = pltpu.bitcast(val.astype(jnp.bfloat16), jnp.uint32)

        def layernorm(blk, ro):
            dsk = tab[T_DSK]
            dsk16 = jnp.concatenate([dsk, dsk], axis=0)
            for g in range(G):
                for j in range(4):
                    los, his = [], []
                    for c in range(NC):
                        w = x32[blk, c, pl.ds(g * 32 + j, 8, stride=4), :]
                        los.append(pltpu.bitcast(w << 16, jnp.float32))
                        his.append(pltpu.bitcast(w & jnp.uint32(0xFFFF0000), jnp.float32))
                    x16 = jnp.concatenate([jnp.concatenate(los, axis=1),
                                           jnp.concatenate(his, axis=1)], axis=0)
                    m = jnp.sum(x16, axis=-1, keepdims=True) * (1.0 / D)
                    xc = x16 - m
                    v = jnp.sum(xc * xc, axis=-1, keepdims=True) * (1.0 / D)
                    r0 = ro + g * 64 + j * 16
                    xnf = xc * lax.rsqrt(v + EPS)
                    st16(xn_s, r0, slice(None), xnf)
                    base_s[pl.ds(r0, 16), :] = x16 + xnf * dsk16

        def dsk_table():
            dsk = pv[3][...].astype(jnp.float32).reshape(1, D)
            tab[T_DSK] = jnp.broadcast_to(dsk, (8, D))

        def build_tables():
            lre = pv[0][...].astype(jnp.float32).reshape(1, P)
            lim = pv[1][...].astype(jnp.float32).reshape(1, P)
            ldt = pv[2][...].astype(jnp.float32).reshape(1, P)
            lre = jnp.broadcast_to(lre, (8, P))
            lim = jnp.broadcast_to(lim, (8, P))
            ldt = jnp.broadcast_to(ldt, (8, P))
            dt = _bf(jnp.exp(ldt))
            mag = jnp.exp(dt * lre)
            ang = dt * lim
            ar = mag * jnp.cos(ang)
            ai = mag * jnp.sin(ang)
            nr, ni = ar - 1.0, ai
            big = jnp.abs(lre) >= jnp.abs(lim)
            num = jnp.where(big, lim, lre)
            den = jnp.where(big, lre, lim)
            rat = num / den
            dd = den + num * rat
            cr = jnp.where(big, nr + ni * rat, nr * rat + ni) / dd
            ci = jnp.where(big, ni - nr * rat, ni * rat - nr) / dd
            cr = 2.0 * cr
            ci = 2.0 * ci
            tab[T_CR] = cr
            tab[T_CI] = ci
            tab[T_NCR] = -cr
            tab[T_A] = ar
            tab[T_A + 1] = ai
            pr, pi = ar, ai
            for _ in range(3):
                pr, pi = pr * pr - pi * pi, 2.0 * pr * pi
            sub = lax.broadcasted_iota(jnp.int32, (8, P), 0)
            for q, sh in enumerate((1, 2, 4)):
                tab[T_T + 2 * q] = jnp.where(sub >= sh, pr, 0.0)
                tab[T_T + 2 * q + 1] = jnp.where(sub >= sh, pi, 0.0)
                pr, pi = pr * pr - pi * pi, 2.0 * pr * pi

        def scan(ro, ng):
            sub = lax.broadcasted_iota(jnp.int32, (8, 128), 0)
            last = sub == 7
            for c in range(NC):
                ln = pl.ds(c * 128, 128)
                T = lambda idx: tab[idx, :, ln]
                hr = hst[0, :, ln]
                hi = hst[1, :, ln]
                def B(g, k):
                    r0 = ro + g * 64 + k * 8
                    return (bu_s[pl.ds(r0, 8), pl.ds(c * 128, 128)],
                            bu_s[pl.ds(r0, 8), pl.ds(P + c * 128, 128)])
                for g in range(ng):
                    er, ei = B(g, 0)
                    for k in range(1, 8):
                        br, bi = B(g, k)
                        er, ei = _cmac(br, bi, T(T_A), T(T_A + 1), er, ei)
                    cr_ = pltpu.roll(jnp.where(last, hr, er), 1, 0)
                    ci_ = pltpu.roll(jnp.where(last, hi, ei), 1, 0)
                    for q, sh in enumerate((1, 2, 4)):
                        cr_, ci_ = _cmac(cr_, ci_, T(T_T + 2 * q), T(T_T + 2 * q + 1),
                                         pltpu.roll(cr_, sh, 0), pltpu.roll(ci_, sh, 0))
                    hr, hi = cr_, ci_
                    for j in range(4):
                        br, bi = B(g, 2 * j)
                        h0r, h0i = _cmac(br, bi, T(T_A), T(T_A + 1), hr, hi)
                        br, bi = B(g, 2 * j + 1)
                        hr, hi = _cmac(br, bi, T(T_A), T(T_A + 1), h0r, h0i)
                        r0 = ro + g * 64 + j * 16
                        st16(h_s, r0, pl.ds(c * 128, 128), jnp.concatenate([h0r, hr], axis=0))
                        st16(h_s, r0, pl.ds(P + c * 128, 128), jnp.concatenate([h0i, hi], axis=0))
                hst[0, :, ln] = hr
                hst[1, :, ln] = hi

        def fold_c():
            c2r = jnp.concatenate([tab[T_CR], tab[T_CR]], axis=0)
            c2i = jnp.concatenate([tab[T_CI], tab[T_CI]], axis=0)
            nc2r = jnp.concatenate([tab[T_NCR], tab[T_NCR]], axis=0)
            for r in range(D // 16):
                rows = pl.ds(r * 16, 16)
                cre = ccat[rows, pl.ds(0, P)].astype(jnp.float32)
                cim = ccat[rows, pl.ds(P, P)].astype(jnp.float32)
                ccat[rows, pl.ds(0, P)] = (cre * c2r - cim * c2i).astype(jnp.bfloat16)
                ccat[rows, pl.ds(P, P)] = (cim * nc2r - cre * c2i).astype(jnp.bfloat16)

        def swiglu(g, u):
            hg = 0.5 * g
            return (hg * u) * (1.0 + jnp.tanh(hg))

        def cproj_col(blk, slot, ro, c):
            yc = yp_s[pl.ds(ro, TL), pl.ds(c * 128, 128)] + _dot(
                ld16(h_s, ro, TL), ccat[pl.ds(c * 128, 128), :], NT_DIMS)
            for g in range(G):
                for k in range(8):
                    r0 = g * 64 + k * 8
                    obuf[slot, c, pl.ds(g * 64 + k, 8, stride=8), :] = yc[r0:r0 + 8, :]
            o_copy(slot, blk, c).start()

        def cproj_out(blk, slot, ro):
            for c in range(NC):
                cproj_col(blk, slot, ro, c)

        def bu_part(ro, nr, t0, t1):
            rows = pl.ds(ro, nr)
            cols = pl.ds(t0 * 128, (t1 - t0) * 128)
            bu_s[rows, cols] = _dot(ld16(xn_s, ro, nr), bcat[cols, :], NT_DIMS)

        def gu_part(ro, ci):
            rows = pl.ds(ro, TL)
            if ci < NGU:
                t0, n = gu_chunks[ci]
                r, d0, a0 = n * 128, 2 * t0 * 128, t0 * 128
            else:
                r, d0, a0 = FT, 2 * FM, FM
            gu = _dot(ld16(xn_s, ro, TL), w13[pl.ds(d0, 2 * r), :], NT_DIMS)
            st16(act_s, ro, pl.ds(a0, r), swiglu(gu[:, :r], gu[:, r:]))

        def down(ro):
            rows = pl.ds(ro, TL)
            yp_s[rows, :] = base_s[rows, :] + _dot(ld16(act_s, ro, TL), w2v[...], NN_DIMS)

        start(x_copies(0))
        start(p_copies())
        start(b_copies(0))
        start(x_copies(1))
        for k in range(1, NBS - 1):
            start(b_copies(k))
        for k in range(NWG):
            start(group_copies(k))
        for blk in range(2, NS):
            start(x_copies(blk))
        hst[...] = jnp.zeros(hst.shape, jnp.float32)
        wait(x_copies(0) + p_copies())
        dsk_table()
        layernorm(0, 0)
        wait(b_copies(0) + x_copies(1))
        bu_part(0, TL, bb[0], bb[1])
        layernorm(1, TL)
        bu_part(TL, TL, bb[0], bb[1])
        for k in range(1, NBS):
            wait(b_copies(k) if k < NBS - 1 else group_copies(0))
            if k == 1:
                build_tables()
            bu_part(0, TL, bb[k], bb[k + 1])
            bu_part(TL, TL, bb[k], bb[k + 1])
        scan(0, 2 * G)
        for ci in range(NGU + 1):
            if ci > 0 and ci in wb:
                wait(group_copies(wb.index(ci)))
            gu_part(0, ci)
            gu_part(TL, ci)
        down(0)
        down(TL)
        fold_c()
        cproj_out(0, 0, 0)
        for blk in range(2, NS):
            wait(x_copies(blk))

        def body(i, carry):
            slot = (i - 1) % 2

            @pl.when(i >= 3)
            def _():
                for c in range(NC):
                    o_copy(slot, jnp.minimum(i - 3, NS - 1), c).wait()

            pb = jnp.minimum(i - 1, NS - 1)
            layernorm(jnp.minimum(i, NS - 1), TL)
            if stagger == 0:
                cproj_out(pb, slot, TL)
                bu_part(TL, TL, 0, 2 * NC)
            elif stagger == 1:
                H = TL // 2
                for c in range(3):
                    cproj_col(pb, slot, TL, c)
                bu_part(TL, H, 0, 2 * NC)
                for c in range(3, NC):
                    cproj_col(pb, slot, TL, c)
                bu_part(TL + H, H, 0, 2 * NC)
            scan(TL, G)
            for ci in range(NGU + 1):
                gu_part(TL, ci)
            down(TL)
            return carry

        lax.fori_loop(2, NS + extra, body, 0)

        slot = (NS + extra - 1) % 2
        for c in range(NC):
            o_copy(slot, NS - 3, c).wait()
        cproj_out(NS - 1, slot, TL)
        for c in range(NC):
            o_copy(1 - slot, NS - 2, c).wait()
        for c in range(NC):
            o_copy(slot, NS - 1, c).wait()

    scratch = [
        pltpu.VMEM((NS, NC, TL, 128), jnp.bfloat16),
        pltpu.VMEM((P,), jnp.bfloat16),
        pltpu.VMEM((P,), jnp.bfloat16),
        pltpu.VMEM((P,), jnp.bfloat16),
        pltpu.VMEM((P,), jnp.bfloat16),
        pltpu.VMEM((2 * P, D), jnp.bfloat16),
        pltpu.VMEM((2 * F, D), jnp.bfloat16),
        pltpu.VMEM((D, 2 * P), jnp.bfloat16),
        pltpu.VMEM((F, D), jnp.bfloat16),
        pltpu.VMEM((N_TAB, 8, P), jnp.float32),
        pltpu.VMEM((2, 8, P), jnp.float32),
        pltpu.VMEM((TL, D), jnp.uint32),
        pltpu.VMEM((2 * TL, D), jnp.float32),
        pltpu.VMEM((2 * TL, D), jnp.float32),
        pltpu.VMEM((TL, 2 * P), jnp.uint32),
        pltpu.VMEM((TL, F), jnp.uint32),
        pltpu.VMEM((2, NC, TL, 128), jnp.float32),
        pltpu.VMEM((2 * TL, 2 * P), jnp.float32),
        pltpu.SemaphoreType.DMA((N_SEM,)),
        pltpu.SemaphoreType.DMA((2,)),
    ]

    @jax.jit
    def fn(A_x, A_Lambda_re, A_Lambda_im, A_B_re, A_B_im, A_C_re, A_C_im, A_log_dt, A_Dskip,
           B_x, B_w1, B_w3, B_w2):
        hbm = pl.BlockSpec(memory_space=pltpu.HBM)
        return pl.pallas_call(
            kernel,
            in_specs=[hbm] * 12,
            out_specs=hbm,
            out_shape=jax.ShapeDtypeStruct((1, L, D), jnp.float32),
            scratch_shapes=scratch,
            compiler_params=pltpu.CompilerParams(
                vmem_limit_bytes=100 * 1024 * 1024),
        )(A_x, A_Lambda_re, A_Lambda_im, A_B_re, A_B_im, A_C_re, A_C_im, A_log_dt, A_Dskip,
          B_w1.T, B_w3.T, B_w2)

    return fn


_impl = make_kernel(TL=256, stagger=1)


@jax.jit
def pallas_parallel_sum__ssm_conv_s5__glu_gated_swiglu__prompt_kernel(
    A_x: jax.Array,
    A_Lambda_re: jax.Array,
    A_Lambda_im: jax.Array,
    A_B_re: jax.Array,
    A_B_im: jax.Array,
    A_C_re: jax.Array,
    A_C_im: jax.Array,
    A_log_dt: jax.Array,
    A_Dskip: jax.Array,
    B_x: jax.Array,
    B_w1: jax.Array,
    B_w3: jax.Array,
    B_w2: jax.Array,
):
    return _impl(A_x, A_Lambda_re, A_Lambda_im, A_B_re, A_B_im, A_C_re, A_C_im, A_log_dt,
                 A_Dskip, B_x, B_w1, B_w3, B_w2)
```

```python
import jax
import jax.numpy as jnp
from jax import lax
import jax.experimental.pallas as pl
import jax.experimental.pallas.tpu as pltpu

L, D, P, F = 2048, 640, 640, 1728
NC = D // 128
FM = (F // 128) * 128
FT = F - FM
NFT = FM // 128
EPS = 1e-5

TL = 256
NS = L // TL
G = TL // 64

NT_DIMS = (((1,), (1,)), ((), ()))
NN_DIMS = (((1,), (0,)), ((), ()))

T_CR, T_CI, T_NCR, T_DSK = 0, 1, 2, 3
T_A = 4
T_T = 6
N_TAB = 12

GU_CHUNKS = tuple((t, min(2, NFT - t)) for t in range(0, NFT, 2))
NGU = len(GU_CHUNKS)
WB = (0, 1, 5, NGU + 1)
NWG = len(WB) - 1
BB = (0, 2, 6, 2 * NC)
NBS = len(BB) - 1

S_X0 = 0
S_B = 1
S_W = S_B + NBS - 1
S_XR = S_W + NWG
S_X1 = S_XR + 1
N_SEM = S_X1 + 1


def _cmac(xr, xi, ar, ai, yr, yi):
    return xr + ar * yr - ai * yi, xi + ar * yi + ai * yr


def _dot(a, b, dims):
    return lax.dot_general(a, b, dims, preferred_element_type=jnp.float32)


def _wgroup_of(ci):
    return [k for k in range(NWG) if WB[k] <= ci < WB[k + 1]][0]


def _kernel(x_hbm, lre_hbm, lim_hbm, bre_hbm, bim_hbm, cre_hbm, cim_hbm, ldt_hbm, dsk_hbm,
            w1t_hbm, w3t_hbm, w2_hbm, o_hbm,
            xs, pv0, pv1, pv2, pv3, bcat, w13, ccat, w2v, tab, hst,
            xn_s, base_s, yp_s, h_s, act_s, obuf, bu_s, st_s, sem, sem_o):
    pv = (pv0, pv1, pv2, pv3)

    def x_copies(blk):
        s = {0: S_X0, 1: S_X1, 2: S_W + NWG - 1}.get(blk, S_XR)
        return [pltpu.make_async_copy(
            x_hbm.at[0, pl.ds(blk * TL, TL), pl.ds(c * 128, 128)],
            xs.at[blk, c], sem.at[s]) for c in range(NC)]

    def p_copies(which):
        srcs = (lre_hbm, lim_hbm, ldt_hbm, dsk_hbm)
        return [pltpu.make_async_copy(srcs[k], pv[k], sem.at[S_X0 if k == 3 else S_B + 1])
                for k in which]

    def b_copies(k):
        r0, r1 = BB[k] * 128, BB[k + 1] * 128
        cps = []
        for src, o in ((bre_hbm, 0), (bim_hbm, P)):
            a, b = max(r0, o), min(r1, o + P)
            if a < b:
                cps.append(pltpu.make_async_copy(src.at[pl.ds(a - o, b - a), :],
                                                 bcat.at[pl.ds(a, b - a), :], sem.at[S_B + k]))
        return cps

    def gu_geom(ci):
        if ci == NGU:
            return FT, 2 * FM, FM
        t0, n = GU_CHUNKS[ci]
        return n * 128, 2 * t0 * 128, t0 * 128

    def w13_copies(ci):
        r, d0, s0 = gu_geom(ci)
        s = sem.at[S_W + _wgroup_of(ci)]
        return [pltpu.make_async_copy(w1t_hbm.at[pl.ds(s0, r), :], w13.at[pl.ds(d0, r), :], s),
                pltpu.make_async_copy(w3t_hbm.at[pl.ds(s0, r), :], w13.at[pl.ds(d0 + r, r), :], s)]

    def group_copies(k):
        cps = b_copies(NBS - 1) if k == 0 else []
        for ci in range(WB[k], WB[k + 1]):
            cps += w13_copies(ci)
        if k == NWG - 1:
            s = sem.at[S_W + k]
            cps += [pltpu.make_async_copy(w2_hbm, w2v, s),
                    pltpu.make_async_copy(cre_hbm, ccat.at[:, pl.ds(0, P)], s),
                    pltpu.make_async_copy(cim_hbm, ccat.at[:, pl.ds(P, P)], s)]
            cps += x_copies(2)
        return cps

    def o_copy(slot, blk, c, g0=0, ng=G):
        return pltpu.make_async_copy(
            obuf.at[slot, c, pl.ds(g0 * 64, ng * 64), :],
            o_hbm.at[0, pl.ds(blk * TL + g0 * 64, ng * 64), pl.ds(c * 128, 128)],
            sem_o.at[slot])

    def start(cps):
        for cp in cps:
            cp.start()

    def wait(cps):
        for cp in cps:
            cp.wait()

    def ld16(ref, r0, nr, cols=slice(None)):
        return pltpu.bitcast(ref[pl.ds(r0 // 2, nr // 2), cols], jnp.bfloat16)

    def st16(ref, r0, cols, val):
        ref[pl.ds(r0 // 2, val.shape[0] // 2), cols] = pltpu.bitcast(
            val.astype(jnp.bfloat16), jnp.uint32)

    x32 = xs.bitcast(jnp.uint32)

    def load_x16(blk, g, j):
        los, his = [], []
        for c in range(NC):
            w = x32[blk, c, pl.ds(g * 32 + j, 8, stride=4), :]
            los.append(pltpu.bitcast(w << 16, jnp.float32))
            his.append(pltpu.bitcast(w & jnp.uint32(0xFFFF0000), jnp.float32))
        return jnp.concatenate([jnp.concatenate(los, axis=1),
                                jnp.concatenate(his, axis=1)], axis=0)

    def stats(x16):
        m = jnp.sum(x16, axis=-1, keepdims=True) * (1.0 / D)
        xc = x16 - m
        v = jnp.sum(xc * xc, axis=-1, keepdims=True) * (1.0 / D)
        return m, xc, lax.rsqrt(v + EPS)

    def ln_store(r0, x16, xnf):
        dsk = tab[T_DSK]
        st16(xn_s, r0, slice(None), xnf)
        base_s[pl.ds(r0, 16), :] = x16 + xnf * jnp.concatenate([dsk, dsk], axis=0)

    def layernorm(blk, ro):
        for g in range(G):
            for j in range(4):
                x16 = load_x16(blk, g, j)
                _, xc, r = stats(x16)
                ln_store(ro + g * 64 + j * 16, x16, xc * r)

    def ln_stats(blk):
        for g in range(G):
            for j in range(4):
                m, _, r = stats(load_x16(blk, g, j))
                r0 = g * 64 + j * 16
                st_s[0, pl.ds(r0, 16), :] = jnp.broadcast_to(m, (16, 128))
                st_s[1, pl.ds(r0, 16), :] = jnp.broadcast_to(r, (16, 128))

    def ln_apply(blk, ro):
        for g in range(G):
            for j in range(4):
                x16 = load_x16(blk, g, j)
                r0 = g * 64 + j * 16
                m = jnp.concatenate([st_s[0, pl.ds(r0, 16), :]] * NC, axis=1)
                r = jnp.concatenate([st_s[1, pl.ds(r0, 16), :]] * NC, axis=1)
                ln_store(ro + r0, x16, (x16 - m) * r)

    def row8(ref):
        return jnp.broadcast_to(ref[...].astype(jnp.float32).reshape(1, P), (8, P))

    def build_tables():
        lre, lim, ldt = row8(pv[0]), row8(pv[1]), row8(pv[2])
        dt = jnp.exp(ldt).astype(jnp.bfloat16).astype(jnp.float32)
        mag = jnp.exp(dt * lre)
        ang = dt * lim
        ar = mag * jnp.cos(ang)
        ai = mag * jnp.sin(ang)
        nr, ni = ar - 1.0, ai
        big = jnp.abs(lre) >= jnp.abs(lim)
        num = jnp.where(big, lim, lre)
        den = jnp.where(big, lre, lim)
        rat = num / den
        dd = den + num * rat
        cr = 2.0 * (jnp.where(big, nr + ni * rat, nr * rat + ni) / dd)
        ci = 2.0 * (jnp.where(big, ni - nr * rat, ni * rat - nr) / dd)
        tab[T_CR] = cr
        tab[T_CI] = ci
        tab[T_NCR] = -cr
        tab[T_A] = ar
        tab[T_A + 1] = ai
        pr, pi = ar, ai
        for _ in range(3):
            pr, pi = pr * pr - pi * pi, 2.0 * pr * pi
        sub = lax.broadcasted_iota(jnp.int32, (8, P), 0)
        for q, sh in enumerate((1, 2, 4)):
            tab[T_T + 2 * q] = jnp.where(sub >= sh, pr, 0.0)
            tab[T_T + 2 * q + 1] = jnp.where(sub >= sh, pi, 0.0)
            pr, pi = pr * pr - pi * pi, 2.0 * pr * pi

    def fold_c():
        c2r = jnp.concatenate([tab[T_CR], tab[T_CR]], axis=0)
        c2i = jnp.concatenate([tab[T_CI], tab[T_CI]], axis=0)
        nc2r = jnp.concatenate([tab[T_NCR], tab[T_NCR]], axis=0)
        for r in range(D // 16):
            rows = pl.ds(r * 16, 16)
            cre = ccat[rows, pl.ds(0, P)].astype(jnp.float32)
            cim = ccat[rows, pl.ds(P, P)].astype(jnp.float32)
            ccat[rows, pl.ds(0, P)] = (cre * c2r - cim * c2i).astype(jnp.bfloat16)
            ccat[rows, pl.ds(P, P)] = (cim * nc2r - cre * c2i).astype(jnp.bfloat16)

    def scan(ro, ng):
        last = lax.broadcasted_iota(jnp.int32, (8, 128), 0) == 7
        for c in range(NC):
            ln = pl.ds(c * 128, 128)
            hr = hst[0, :, ln]
            hi = hst[1, :, ln]

            def T(idx):
                return tab[idx, :, ln]

            def B(g, k):
                r0 = ro + g * 64 + k * 8
                return (bu_s[pl.ds(r0, 8), pl.ds(c * 128, 128)],
                        bu_s[pl.ds(r0, 8), pl.ds(P + c * 128, 128)])

            for g in range(ng):
                er, ei = B(g, 0)
                for k in range(1, 8):
                    er, ei = _cmac(*B(g, k), T(T_A), T(T_A + 1), er, ei)
                hr = pltpu.roll(jnp.where(last, hr, er), 1, 0)
                hi = pltpu.roll(jnp.where(last, hi, ei), 1, 0)
                for q, sh in enumerate((1, 2, 4)):
                    hr, hi = _cmac(hr, hi, T(T_T + 2 * q), T(T_T + 2 * q + 1),
                                   pltpu.roll(hr, sh, 0), pltpu.roll(hi, sh, 0))
                for j in range(4):
                    h0r, h0i = _cmac(*B(g, 2 * j), T(T_A), T(T_A + 1), hr, hi)
                    hr, hi = _cmac(*B(g, 2 * j + 1), T(T_A), T(T_A + 1), h0r, h0i)
                    r0 = ro + g * 64 + j * 16
                    st16(h_s, r0, pl.ds(c * 128, 128), jnp.concatenate([h0r, hr], axis=0))
                    st16(h_s, r0, pl.ds(P + c * 128, 128), jnp.concatenate([h0i, hi], axis=0))
            hst[0, :, ln] = hr
            hst[1, :, ln] = hi

    def bu_part(ro, t0, t1):
        cols = pl.ds(t0 * 128, (t1 - t0) * 128)
        bu_s[pl.ds(ro, TL), cols] = _dot(ld16(xn_s, ro, TL), bcat[cols, :], NT_DIMS)

    def gu_part(ro, ci):
        r, d0, a0 = gu_geom(ci)
        gu = _dot(ld16(xn_s, ro, TL), w13[pl.ds(d0, 2 * r), :], NT_DIMS)
        hg = 0.5 * gu[:, :r]
        st16(act_s, ro, pl.ds(a0, r), (hg * gu[:, r:]) * (1.0 + jnp.tanh(hg)))

    def down_main(ro):
        rows = pl.ds(ro, TL)
        yp_s[rows, :] = base_s[rows, :] + _dot(ld16(act_s, ro, TL, pl.ds(0, FM)),
                                               w2v[pl.ds(0, FM), :], NN_DIMS)

    def finish_col(blk, slot, ro, c, msplit=1, gdma=False):
        cols = pl.ds(c * 128, 128)
        q = TL // msplit
        tail = [_dot(ld16(act_s, ro + k * q, q, pl.ds(FM, FT)), w2v[pl.ds(FM, FT), cols], NN_DIMS)
                for k in range(msplit)]
        yc = yp_s[pl.ds(ro, TL), cols] + jnp.concatenate(tail, axis=0)
        yc = yc + _dot(ld16(h_s, ro, TL), ccat[cols, :], NT_DIMS)
        for g in range(G):
            for k in range(8):
                r0 = g * 64 + k * 8
                obuf[slot, c, pl.ds(g * 64 + k, 8, stride=8), :] = yc[r0:r0 + 8, :]
            if gdma:
                o_copy(slot, blk, c, g, 1).start()
        if not gdma:
            o_copy(slot, blk, c).start()

    start(x_copies(0) + p_copies((3,)))
    start(x_copies(1))
    start(b_copies(0))
    start(p_copies((0, 1, 2)))
    for k in range(1, NBS - 1):
        start(b_copies(k))
    for k in range(NWG):
        start(group_copies(k))
    for blk in range(3, NS):
        start(x_copies(blk))
    hst[...] = jnp.zeros(hst.shape, jnp.float32)
    wait(x_copies(0) + p_copies((3,)))
    tab[T_DSK] = row8(pv[3])
    layernorm(0, 0)
    wait(x_copies(1))
    layernorm(1, TL)
    for k in range(NBS):
        wait(b_copies(k) if k < NBS - 1 else group_copies(0))
        if k == 1:
            wait(p_copies((0, 1, 2)))
            build_tables()
        bu_part(0, BB[k], BB[k + 1])
        bu_part(TL, BB[k], BB[k + 1])
    scan(0, 2 * G)
    for ci in range(NGU + 1):
        if ci > 0 and ci in WB:
            wait(group_copies(WB.index(ci)))
        gu_part(0, ci)
        gu_part(TL, ci)
    down_main(0)
    down_main(TL)
    fold_c()
    for c in range(NC):
        finish_col(0, 0, 0, c, msplit=4 if c < 3 else 1)
    ln_stats(2)
    for blk in range(3, NS):
        wait(x_copies(blk))

    def body(i, carry):
        slot = (i - 1) % 2

        @pl.when(i >= 3)
        def _():
            for c in range(NC):
                o_copy(slot, i - 3, c).wait()

        ln_apply(i, TL)
        for c in range(NC):
            finish_col(i - 1, slot, TL, c)
        for c in range(NC):
            bu_part(TL, c, c + 1)
            bu_part(TL, NC + c, NC + c + 1)
        scan(TL, G)
        for ci in range(NGU + 1):
            gu_part(TL, ci)
        down_main(TL)
        ln_stats(jnp.minimum(i + 1, NS - 1))
        return carry

    lax.fori_loop(2, NS, body, 0)

    slot = (NS - 1) % 2
    for c in range(NC):
        o_copy(slot, NS - 3, c).wait()
    for c in range(NC):
        finish_col(NS - 1, slot, TL, c, gdma=(c == NC - 1))
    for c in range(NC):
        o_copy(1 - slot, NS - 2, c).wait()
    for c in range(NC - 1):
        o_copy(slot, NS - 1, c).wait()
    for g in range(G):
        o_copy(slot, NS - 1, NC - 1, g, 1).wait()


_SCRATCH = [
    pltpu.VMEM((NS, NC, TL, 128), jnp.bfloat16),
    pltpu.VMEM((P,), jnp.bfloat16),
    pltpu.VMEM((P,), jnp.bfloat16),
    pltpu.VMEM((P,), jnp.bfloat16),
    pltpu.VMEM((D,), jnp.bfloat16),
    pltpu.VMEM((2 * P, D), jnp.bfloat16),
    pltpu.VMEM((2 * F, D), jnp.bfloat16),
    pltpu.VMEM((D, 2 * P), jnp.bfloat16),
    pltpu.VMEM((F, D), jnp.bfloat16),
    pltpu.VMEM((N_TAB, 8, P), jnp.float32),
    pltpu.VMEM((2, 8, P), jnp.float32),
    pltpu.VMEM((TL, D), jnp.uint32),
    pltpu.VMEM((2 * TL, D), jnp.float32),
    pltpu.VMEM((2 * TL, D), jnp.float32),
    pltpu.VMEM((TL, 2 * P), jnp.uint32),
    pltpu.VMEM((TL, F), jnp.uint32),
    pltpu.VMEM((2, NC, TL, 128), jnp.float32),
    pltpu.VMEM((2 * TL, 2 * P), jnp.float32),
    pltpu.VMEM((2, TL, 128), jnp.float32),
    pltpu.SemaphoreType.DMA((N_SEM,)),
    pltpu.SemaphoreType.DMA((2,)),
]


@jax.jit
def pallas_parallel_sum__ssm_conv_s5__glu_gated_swiglu__prompt_kernel(
    A_x: jax.Array,
    A_Lambda_re: jax.Array,
    A_Lambda_im: jax.Array,
    A_B_re: jax.Array,
    A_B_im: jax.Array,
    A_C_re: jax.Array,
    A_C_im: jax.Array,
    A_log_dt: jax.Array,
    A_Dskip: jax.Array,
    B_x: jax.Array,
    B_w1: jax.Array,
    B_w3: jax.Array,
    B_w2: jax.Array,
):
    del B_x
    hbm = pl.BlockSpec(memory_space=pltpu.HBM)
    return pl.pallas_call(
        _kernel,
        in_specs=[hbm] * 12,
        out_specs=hbm,
        out_shape=jax.ShapeDtypeStruct((1, L, D), jnp.float32),
        scratch_shapes=_SCRATCH,
        compiler_params=pltpu.CompilerParams(
            vmem_limit_bytes=100 * 1024 * 1024,
            disable_bounds_checks=True,
            disable_semaphore_checks=True,
        ),
    )(A_x, A_Lambda_re, A_Lambda_im, A_B_re, A_B_im, A_C_re, A_C_im, A_log_dt, A_Dskip,
      B_w1.T, B_w3.T, B_w2)
```

```python
import jax
import jax.numpy as jnp
from jax import lax
import jax.experimental.pallas as pl
import jax.experimental.pallas.tpu as pltpu

L, D, P, F = 2048, 640, 640, 1728
NC = D // 128
FM = (F // 128) * 128
FT = F - FM
NFT = FM // 128
EPS = 1e-5

TL = 256
NS = L // TL
G = TL // 64

NT_DIMS = (((1,), (1,)), ((), ()))
NN_DIMS = (((1,), (0,)), ((), ()))

T_CR, T_CI, T_NCR, T_DSK = 0, 1, 2, 3
T_A = 4
T_T = 6
N_TAB = 12

GU_CHUNKS = tuple((t, min(2, NFT - t)) for t in range(0, NFT, 2))
NGU = len(GU_CHUNKS)
WB = (0, 1, 5, NGU + 1)
NWG = len(WB) - 1
BB = (0, 2, 6, 2 * NC)
NBS = len(BB) - 1

S_X0 = 0
S_B = 1
S_W = S_B + NBS - 1
S_XR = S_W + NWG
S_X1 = S_XR + 1
N_SEM = S_X1 + 1


def _cmac(xr, xi, ar, ai, yr, yi):
    return xr + ar * yr - ai * yi, xi + ar * yi + ai * yr


def _dot(a, b, dims):
    return lax.dot_general(a, b, dims, preferred_element_type=jnp.float32)


def _wgroup_of(ci):
    return [k for k in range(NWG) if WB[k] <= ci < WB[k + 1]][0]


def _kernel(x_hbm, lre_hbm, lim_hbm, bre_hbm, bim_hbm, cre_hbm, cim_hbm, ldt_hbm, dsk_hbm,
            w1t_hbm, w3t_hbm, w2_hbm, o_hbm,
            xs, pv0, pv1, pv2, pv3, bcat, w13, ccat, w2v, tab, hst,
            xn_s, base_s, yp_s, h_s, act_s, obuf, bu_s, st_s, sem, sem_o):
    pv = (pv0, pv1, pv2, pv3)

    def x_copies(blk):
        s = {0: S_X0, 1: S_X1, 2: S_W + NWG - 1}.get(blk, S_XR)
        return [pltpu.make_async_copy(
            x_hbm.at[0, pl.ds(blk * TL, TL), pl.ds(c * 128, 128)],
            xs.at[blk, c], sem.at[s]) for c in range(NC)]

    def p_copies(which):
        srcs = (lre_hbm, lim_hbm, ldt_hbm, dsk_hbm)
        return [pltpu.make_async_copy(srcs[k], pv[k], sem.at[S_X0 if k == 3 else S_B + 1])
                for k in which]

    def b_copies(k):
        r0, r1 = BB[k] * 128, BB[k + 1] * 128
        cps = []
        for src, o in ((bre_hbm, 0), (bim_hbm, P)):
            a, b = max(r0, o), min(r1, o + P)
            if a < b:
                cps.append(pltpu.make_async_copy(src.at[pl.ds(a - o, b - a), :],
                                                 bcat.at[pl.ds(a, b - a), :], sem.at[S_B + k]))
        return cps

    def gu_geom(ci):
        if ci == NGU:
            return FT, 2 * FM, FM
        t0, n = GU_CHUNKS[ci]
        return n * 128, 2 * t0 * 128, t0 * 128

    def w13_copies(ci):
        r, d0, s0 = gu_geom(ci)
        s = sem.at[S_W + _wgroup_of(ci)]
        return [pltpu.make_async_copy(w1t_hbm.at[pl.ds(s0, r), :], w13.at[pl.ds(d0, r), :], s),
                pltpu.make_async_copy(w3t_hbm.at[pl.ds(s0, r), :], w13.at[pl.ds(d0 + r, r), :], s)]

    def group_copies(k):
        cps = b_copies(NBS - 1) if k == 0 else []
        for ci in range(WB[k], WB[k + 1]):
            cps += w13_copies(ci)
        if k == NWG - 1:
            s = sem.at[S_W + k]
            cps += [pltpu.make_async_copy(w2_hbm, w2v, s),
                    pltpu.make_async_copy(cre_hbm, ccat.at[:, pl.ds(0, P)], s),
                    pltpu.make_async_copy(cim_hbm, ccat.at[:, pl.ds(P, P)], s)]
            cps += x_copies(2)
        return cps

    def o_copy(blk, c, g0=0, ng=G):
        return pltpu.make_async_copy(
            obuf.at[blk, c, pl.ds(g0 * 64, ng * 64), :],
            o_hbm.at[0, pl.ds(blk * TL + g0 * 64, ng * 64), pl.ds(c * 128, 128)],
            sem_o.at[0])

    def start(cps):
        for cp in cps:
            cp.start()

    def wait(cps):
        for cp in cps:
            cp.wait()

    def ld16(ref, r0, nr, cols=slice(None)):
        return pltpu.bitcast(ref[pl.ds(r0 // 2, nr // 2), cols], jnp.bfloat16)

    def st16(ref, r0, cols, val):
        ref[pl.ds(r0 // 2, val.shape[0] // 2), cols] = pltpu.bitcast(
            val.astype(jnp.bfloat16), jnp.uint32)

    x32 = xs.bitcast(jnp.uint32)

    def load_x16(blk, g, j):
        los, his = [], []
        for c in range(NC):
            w = x32[blk, c, pl.ds(g * 32 + j, 8, stride=4), :]
            los.append(pltpu.bitcast(w << 16, jnp.float32))
            his.append(pltpu.bitcast(w & jnp.uint32(0xFFFF0000), jnp.float32))
        return jnp.concatenate([jnp.concatenate(los, axis=1),
                                jnp.concatenate(his, axis=1)], axis=0)

    def stats(x16):
        m = jnp.sum(x16, axis=-1, keepdims=True) * (1.0 / D)
        xc = x16 - m
        v = jnp.sum(xc * xc, axis=-1, keepdims=True) * (1.0 / D)
        return m, xc, lax.rsqrt(v + EPS)

    def ln_store(r0, x16, xnf):
        dsk = tab[T_DSK]
        st16(xn_s, r0, slice(None), xnf)
        base_s[pl.ds(r0, 16), :] = x16 + xnf * jnp.concatenate([dsk, dsk], axis=0)

    def layernorm(blk, ro):
        for g in range(G):
            for j in range(4):
                x16 = load_x16(blk, g, j)
                _, xc, r = stats(x16)
                ln_store(ro + g * 64 + j * 16, x16, xc * r)

    def ln_stats(blk):
        for g in range(G):
            for j in range(4):
                m, _, r = stats(load_x16(blk, g, j))
                r0 = g * 64 + j * 16
                st_s[0, pl.ds(r0, 16), :] = jnp.broadcast_to(m, (16, 128))
                st_s[1, pl.ds(r0, 16), :] = jnp.broadcast_to(r, (16, 128))

    def ln_apply(blk, ro):
        for g in range(G):
            for j in range(4):
                x16 = load_x16(blk, g, j)
                r0 = g * 64 + j * 16
                m = jnp.concatenate([st_s[0, pl.ds(r0, 16), :]] * NC, axis=1)
                r = jnp.concatenate([st_s[1, pl.ds(r0, 16), :]] * NC, axis=1)
                ln_store(ro + r0, x16, (x16 - m) * r)

    def row8(ref):
        return jnp.broadcast_to(ref[...].astype(jnp.float32).reshape(1, P), (8, P))

    def build_tables():
        lre, lim, ldt = row8(pv[0]), row8(pv[1]), row8(pv[2])
        dt = jnp.exp(ldt).astype(jnp.bfloat16).astype(jnp.float32)
        mag = jnp.exp(dt * lre)
        ang = dt * lim
        ar = mag * jnp.cos(ang)
        ai = mag * jnp.sin(ang)
        nr, ni = ar - 1.0, ai
        big = jnp.abs(lre) >= jnp.abs(lim)
        num = jnp.where(big, lim, lre)
        den = jnp.where(big, lre, lim)
        rat = num / den
        dd = den + num * rat
        cr = 2.0 * (jnp.where(big, nr + ni * rat, nr * rat + ni) / dd)
        ci = 2.0 * (jnp.where(big, ni - nr * rat, ni * rat - nr) / dd)
        tab[T_CR] = cr
        tab[T_CI] = ci
        tab[T_NCR] = -cr
        tab[T_A] = ar
        tab[T_A + 1] = ai
        pr, pi = ar, ai
        for _ in range(3):
            pr, pi = pr * pr - pi * pi, 2.0 * pr * pi
        sub = lax.broadcasted_iota(jnp.int32, (8, P), 0)
        for q, sh in enumerate((1, 2, 4)):
            tab[T_T + 2 * q] = jnp.where(sub >= sh, pr, 0.0)
            tab[T_T + 2 * q + 1] = jnp.where(sub >= sh, pi, 0.0)
            pr, pi = pr * pr - pi * pi, 2.0 * pr * pi

    def fold_c():
        c2r = jnp.concatenate([tab[T_CR], tab[T_CR]], axis=0)
        c2i = jnp.concatenate([tab[T_CI], tab[T_CI]], axis=0)
        nc2r = jnp.concatenate([tab[T_NCR], tab[T_NCR]], axis=0)
        for r in range(D // 16):
            rows = pl.ds(r * 16, 16)
            cre = ccat[rows, pl.ds(0, P)].astype(jnp.float32)
            cim = ccat[rows, pl.ds(P, P)].astype(jnp.float32)
            ccat[rows, pl.ds(0, P)] = (cre * c2r - cim * c2i).astype(jnp.bfloat16)
            ccat[rows, pl.ds(P, P)] = (cim * nc2r - cre * c2i).astype(jnp.bfloat16)

    def scan(ro, ng):
        last = lax.broadcasted_iota(jnp.int32, (8, 128), 0) == 7
        for c in range(NC):
            ln = pl.ds(c * 128, 128)
            hr = hst[0, :, ln]
            hi = hst[1, :, ln]

            def T(idx):
                return tab[idx, :, ln]

            def B(g, k):
                r0 = ro + g * 64 + k * 8
                return (bu_s[pl.ds(r0, 8), pl.ds(c * 128, 128)],
                        bu_s[pl.ds(r0, 8), pl.ds(P + c * 128, 128)])

            for g in range(ng):
                er, ei = B(g, 0)
                for k in range(1, 8):
                    er, ei = _cmac(*B(g, k), T(T_A), T(T_A + 1), er, ei)
                hr = pltpu.roll(jnp.where(last, hr, er), 1, 0)
                hi = pltpu.roll(jnp.where(last, hi, ei), 1, 0)
                for q, sh in enumerate((1, 2, 4)):
                    hr, hi = _cmac(hr, hi, T(T_T + 2 * q), T(T_T + 2 * q + 1),
                                   pltpu.roll(hr, sh, 0), pltpu.roll(hi, sh, 0))
                for j in range(4):
                    h0r, h0i = _cmac(*B(g, 2 * j), T(T_A), T(T_A + 1), hr, hi)
                    hr, hi = _cmac(*B(g, 2 * j + 1), T(T_A), T(T_A + 1), h0r, h0i)
                    r0 = ro + g * 64 + j * 16
                    st16(h_s, r0, pl.ds(c * 128, 128), jnp.concatenate([h0r, hr], axis=0))
                    st16(h_s, r0, pl.ds(P + c * 128, 128), jnp.concatenate([h0i, hi], axis=0))
            hst[0, :, ln] = hr
            hst[1, :, ln] = hi

    def bu_part(ro, t0, t1):
        cols = pl.ds(t0 * 128, (t1 - t0) * 128)
        bu_s[pl.ds(ro, TL), cols] = _dot(ld16(xn_s, ro, TL), bcat[cols, :], NT_DIMS)

    def gu_part(ro, ci):
        r, d0, a0 = gu_geom(ci)
        gu = _dot(ld16(xn_s, ro, TL), w13[pl.ds(d0, 2 * r), :], NT_DIMS)
        hg = 0.5 * gu[:, :r]
        st16(act_s, ro, pl.ds(a0, r), (hg * gu[:, r:]) * (1.0 + jnp.tanh(hg)))

    def down_main(ro):
        rows = pl.ds(ro, TL)
        yp_s[rows, :] = base_s[rows, :] + _dot(ld16(act_s, ro, TL, pl.ds(0, FM)),
                                               w2v[pl.ds(0, FM), :], NN_DIMS)

    def finish_col(blk, ro, c, msplit=1, gdma=False):
        cols = pl.ds(c * 128, 128)
        q = TL // msplit
        tail = [_dot(ld16(act_s, ro + k * q, q, pl.ds(FM, FT)), w2v[pl.ds(FM, FT), cols], NN_DIMS)
                for k in range(msplit)]
        yc = yp_s[pl.ds(ro, TL), cols] + jnp.concatenate(tail, axis=0)
        yc = yc + _dot(ld16(h_s, ro, TL), ccat[cols, :], NT_DIMS)
        for g in range(G):
            for k in range(8):
                r0 = g * 64 + k * 8
                obuf[blk, c, pl.ds(g * 64 + k, 8, stride=8), :] = yc[r0:r0 + 8, :]
            if gdma:
                o_copy(blk, c, g, 1).start()
        if not gdma:
            o_copy(blk, c).start()

    start(x_copies(0) + p_copies((3,)))
    start(x_copies(1))
    start(b_copies(0))
    start(p_copies((0, 1, 2)))
    for k in range(1, NBS - 1):
        start(b_copies(k))
    for k in range(NWG):
        start(group_copies(k))
    for blk in range(3, NS):
        start(x_copies(blk))
    hst[...] = jnp.zeros(hst.shape, jnp.float32)
    wait(x_copies(0) + p_copies((3,)))
    tab[T_DSK] = row8(pv[3])
    layernorm(0, 0)
    wait(x_copies(1))
    layernorm(1, TL)
    for k in range(NBS):
        wait(b_copies(k) if k < NBS - 1 else group_copies(0))
        if k == 1:
            wait(p_copies((0, 1, 2)))
            build_tables()
        bu_part(0, BB[k], BB[k + 1])
        bu_part(TL, BB[k], BB[k + 1])
    scan(0, 2 * G)
    for ci in range(NGU + 1):
        if ci > 0 and ci in WB:
            wait(group_copies(WB.index(ci)))
        gu_part(0, ci)
        gu_part(TL, ci)
    down_main(0)
    down_main(TL)
    fold_c()
    for c in range(NC):
        finish_col(0, 0, c, msplit=4 if c < 3 else 1)
    ln_stats(2)
    for blk in range(3, NS):
        wait(x_copies(blk))

    def body(i, carry):
        ln_apply(i, TL)
        for c in range(NC):
            finish_col(i - 1, TL, c)
        for c in range(NC):
            bu_part(TL, c, c + 1)
            bu_part(TL, NC + c, NC + c + 1)
        scan(TL, G)
        for ci in range(NGU + 1):
            gu_part(TL, ci)
        down_main(TL)
        ln_stats(jnp.minimum(i + 1, NS - 1))
        return carry

    lax.fori_loop(2, NS, body, 0)

    for c in range(NC):
        finish_col(NS - 1, TL, c, gdma=(c == NC - 1))
    for blk in range(NS):
        for c in range(NC):
            if (blk, c) == (NS - 1, NC - 1):
                for g in range(G):
                    o_copy(blk, c, g, 1).wait()
            else:
                o_copy(blk, c).wait()


_SCRATCH = [
    pltpu.VMEM((NS, NC, TL, 128), jnp.bfloat16),
    pltpu.VMEM((P,), jnp.bfloat16),
    pltpu.VMEM((P,), jnp.bfloat16),
    pltpu.VMEM((P,), jnp.bfloat16),
    pltpu.VMEM((D,), jnp.bfloat16),
    pltpu.VMEM((2 * P, D), jnp.bfloat16),
    pltpu.VMEM((2 * F, D), jnp.bfloat16),
    pltpu.VMEM((D, 2 * P), jnp.bfloat16),
    pltpu.VMEM((F, D), jnp.bfloat16),
    pltpu.VMEM((N_TAB, 8, P), jnp.float32),
    pltpu.VMEM((2, 8, P), jnp.float32),
    pltpu.VMEM((TL, D), jnp.uint32),
    pltpu.VMEM((2 * TL, D), jnp.float32),
    pltpu.VMEM((2 * TL, D), jnp.float32),
    pltpu.VMEM((TL, 2 * P), jnp.uint32),
    pltpu.VMEM((TL, F), jnp.uint32),
    pltpu.VMEM((NS, NC, TL, 128), jnp.float32),
    pltpu.VMEM((2 * TL, 2 * P), jnp.float32),
    pltpu.VMEM((2, TL, 128), jnp.float32),
    pltpu.SemaphoreType.DMA((N_SEM,)),
    pltpu.SemaphoreType.DMA((1,)),
]


@jax.jit
def pallas_parallel_sum__ssm_conv_s5__glu_gated_swiglu__prompt_kernel(
    A_x: jax.Array,
    A_Lambda_re: jax.Array,
    A_Lambda_im: jax.Array,
    A_B_re: jax.Array,
    A_B_im: jax.Array,
    A_C_re: jax.Array,
    A_C_im: jax.Array,
    A_log_dt: jax.Array,
    A_Dskip: jax.Array,
    B_x: jax.Array,
    B_w1: jax.Array,
    B_w3: jax.Array,
    B_w2: jax.Array,
):
    del B_x
    hbm = pl.BlockSpec(memory_space=pltpu.HBM)
    return pl.pallas_call(
        _kernel,
        in_specs=[hbm] * 12,
        out_specs=hbm,
        out_shape=jax.ShapeDtypeStruct((1, L, D), jnp.float32),
        scratch_shapes=_SCRATCH,
        compiler_params=pltpu.CompilerParams(
            vmem_limit_bytes=100 * 1024 * 1024,
            disable_bounds_checks=True,
            disable_semaphore_checks=True,
        ),
    )(A_x, A_Lambda_re, A_Lambda_im, A_B_re, A_B_im, A_C_re, A_C_im, A_log_dt, A_Dskip,
      B_w1.T, B_w3.T, B_w2)
```

```python
import dataclasses

import jax
import jax.numpy as jnp
from jax import lax
import jax.experimental.pallas as pl
import jax.experimental.pallas.tpu as pltpu

L, D, P, F = 2048, 640, 640, 1728
NC = D // 128
FM = (F // 128) * 128
FT = F - FM
NFT = FM // 128
EPS = 1e-5

TL = 256
NS = L // TL
G = TL // 64

NT_DIMS = (((1,), (1,)), ((), ()))
NN_DIMS = (((1,), (0,)), ((), ()))

T_CR, T_CI, T_NCR, T_DSK = 0, 1, 2, 3
T_A = 4
T_T = 6
N_TAB = 12

GU_CHUNKS = tuple((t, min(2, NFT - t)) for t in range(0, NFT, 2))
NGU = len(GU_CHUNKS)
WB = (0, 1, 5, NGU + 1)
NWG = len(WB) - 1
BB = (0, 2, 6, 2 * NC)
NBS = len(BB) - 1

S_X0 = 0
S_B = 1
S_W = S_B + NBS - 1
S_XR = S_W + NWG
S_X1 = S_XR + 1
N_SEM = S_X1 + 1


def _cmac(xr, xi, ar, ai, yr, yi):
    return xr + ar * yr - ai * yi, xi + ar * yi + ai * yr


def _dot(a, b, dims):
    return lax.dot_general(a, b, dims, preferred_element_type=jnp.float32)


def _wgroup_of(ci):
    return [k for k in range(NWG) if WB[k] <= ci < WB[k + 1]][0]


def _kernel(x_hbm, lre_hbm, lim_hbm, bre_hbm, bim_hbm, cre_hbm, cim_hbm, ldt_hbm, dsk_hbm,
            w1t_hbm, w3t_hbm, w2_hbm, o_hbm,
            xs, pv0, pv1, pv2, pv3, bcat, w13, ccat, w2v, tab, hst,
            xn_s, base_s, yp_s, h_s, act_s, obuf, bu_s, st_s, sem, sem_o):
    pv = (pv0, pv1, pv2, pv3)

    def x_copies(blk):
        s = {0: S_X0, 1: S_X1, 2: S_W + NWG - 1}.get(blk, S_XR)
        return [pltpu.make_async_copy(
            x_hbm.at[0, pl.ds(blk * TL, TL), pl.ds(c * 128, 128)],
            xs.at[blk, c], sem.at[s]) for c in range(NC)]

    def p_copies(which):
        srcs = (lre_hbm, lim_hbm, ldt_hbm, dsk_hbm)
        return [pltpu.make_async_copy(srcs[k], pv[k], sem.at[S_X0 if k == 3 else S_B + 1])
                for k in which]

    def b_copies(k):
        r0, r1 = BB[k] * 128, BB[k + 1] * 128
        cps = []
        for src, o in ((bre_hbm, 0), (bim_hbm, P)):
            a, b = max(r0, o), min(r1, o + P)
            if a < b:
                cps.append(pltpu.make_async_copy(src.at[pl.ds(a - o, b - a), :],
                                                 bcat.at[pl.ds(a, b - a), :], sem.at[S_B + k]))
        return cps

    def gu_geom(ci):
        if ci == NGU:
            return FT, 2 * FM, FM
        t0, n = GU_CHUNKS[ci]
        return n * 128, 2 * t0 * 128, t0 * 128

    def w13_copies(ci):
        r, d0, s0 = gu_geom(ci)
        s = sem.at[S_W + _wgroup_of(ci)]
        return [pltpu.make_async_copy(w1t_hbm.at[pl.ds(s0, r), :], w13.at[pl.ds(d0, r), :], s),
                pltpu.make_async_copy(w3t_hbm.at[pl.ds(s0, r), :], w13.at[pl.ds(d0 + r, r), :], s)]

    def group_copies(k):
        cps = b_copies(NBS - 1) if k == 0 else []
        for ci in range(WB[k], WB[k + 1]):
            cps += w13_copies(ci)
        if k == NWG - 1:
            s = sem.at[S_W + k]
            cps += [pltpu.make_async_copy(w2_hbm, w2v, s),
                    pltpu.make_async_copy(cre_hbm, ccat.at[:, pl.ds(0, P)], s),
                    pltpu.make_async_copy(cim_hbm, ccat.at[:, pl.ds(P, P)], s)]
            cps += x_copies(2)
        return cps

    def o_copy(blk, c, g0=0, ng=G):
        return pltpu.make_async_copy(
            obuf.at[blk, c, pl.ds(g0 * 64, ng * 64), :],
            o_hbm.at[0, pl.ds(blk * TL + g0 * 64, ng * 64), pl.ds(c * 128, 128)],
            sem_o.at[0])

    def start(cps):
        for cp in cps:
            cp.start()

    def wait(cps):
        for cp in cps:
            cp.wait()

    def ld16(ref, r0, nr, cols=slice(None)):
        return pltpu.bitcast(ref[pl.ds(r0 // 2, nr // 2), cols], jnp.bfloat16)

    def st16(ref, r0, cols, val):
        ref[pl.ds(r0 // 2, val.shape[0] // 2), cols] = pltpu.bitcast(
            val.astype(jnp.bfloat16), jnp.uint32)

    x32 = xs.bitcast(jnp.uint32)

    def load_x16(blk, g, j):
        los, his = [], []
        for c in range(NC):
            w = x32[blk, c, pl.ds(g * 32 + j, 8, stride=4), :]
            los.append(pltpu.bitcast(w << 16, jnp.float32))
            his.append(pltpu.bitcast(w & jnp.uint32(0xFFFF0000), jnp.float32))
        return jnp.concatenate([jnp.concatenate(los, axis=1),
                                jnp.concatenate(his, axis=1)], axis=0)

    def stats(x16):
        m = jnp.sum(x16, axis=-1, keepdims=True) * (1.0 / D)
        xc = x16 - m
        v = jnp.sum(xc * xc, axis=-1, keepdims=True) * (1.0 / D)
        return m, xc, lax.rsqrt(v + EPS)

    def ln_store(r0, x16, xnf):
        dsk = tab[T_DSK]
        st16(xn_s, r0, slice(None), xnf)
        base_s[pl.ds(r0, 16), :] = x16 + xnf * jnp.concatenate([dsk, dsk], axis=0)

    def layernorm(blk, ro):
        for g in range(G):
            for j in range(4):
                x16 = load_x16(blk, g, j)
                _, xc, r = stats(x16)
                ln_store(ro + g * 64 + j * 16, x16, xc * r)

    def ln_stats(blk):
        for g in range(G):
            for j in range(4):
                m, _, r = stats(load_x16(blk, g, j))
                r0 = g * 64 + j * 16
                st_s[0, pl.ds(r0, 16), :] = jnp.broadcast_to(m, (16, 128))
                st_s[1, pl.ds(r0, 16), :] = jnp.broadcast_to(r, (16, 128))

    def ln_apply(blk, ro):
        for g in range(G):
            for j in range(4):
                x16 = load_x16(blk, g, j)
                r0 = g * 64 + j * 16
                m = jnp.concatenate([st_s[0, pl.ds(r0, 16), :]] * NC, axis=1)
                r = jnp.concatenate([st_s[1, pl.ds(r0, 16), :]] * NC, axis=1)
                ln_store(ro + r0, x16, (x16 - m) * r)

    def row8(ref):
        return jnp.broadcast_to(ref[...].astype(jnp.float32).reshape(1, P), (8, P))

    def build_tables():
        lre, lim, ldt = row8(pv[0]), row8(pv[1]), row8(pv[2])
        dt = jnp.exp(ldt).astype(jnp.bfloat16).astype(jnp.float32)
        mag = jnp.exp(dt * lre)
        ang = dt * lim
        ar = mag * jnp.cos(ang)
        ai = mag * jnp.sin(ang)
        nr, ni = ar - 1.0, ai
        big = jnp.abs(lre) >= jnp.abs(lim)
        num = jnp.where(big, lim, lre)
        den = jnp.where(big, lre, lim)
        rat = num / den
        dd = den + num * rat
        cr = 2.0 * (jnp.where(big, nr + ni * rat, nr * rat + ni) / dd)
        ci = 2.0 * (jnp.where(big, ni - nr * rat, ni * rat - nr) / dd)
        tab[T_CR] = cr
        tab[T_CI] = ci
        tab[T_NCR] = -cr
        tab[T_A] = ar
        tab[T_A + 1] = ai
        pr, pi = ar, ai
        for _ in range(3):
            pr, pi = pr * pr - pi * pi, 2.0 * pr * pi
        sub = lax.broadcasted_iota(jnp.int32, (8, P), 0)
        for q, sh in enumerate((1, 2, 4)):
            tab[T_T + 2 * q] = jnp.where(sub >= sh, pr, 0.0)
            tab[T_T + 2 * q + 1] = jnp.where(sub >= sh, pi, 0.0)
            pr, pi = pr * pr - pi * pi, 2.0 * pr * pi

    def fold_c():
        c2r = jnp.concatenate([tab[T_CR], tab[T_CR]], axis=0)
        c2i = jnp.concatenate([tab[T_CI], tab[T_CI]], axis=0)
        nc2r = jnp.concatenate([tab[T_NCR], tab[T_NCR]], axis=0)
        for r in range(D // 16):
            rows = pl.ds(r * 16, 16)
            cre = ccat[rows, pl.ds(0, P)].astype(jnp.float32)
            cim = ccat[rows, pl.ds(P, P)].astype(jnp.float32)
            ccat[rows, pl.ds(0, P)] = (cre * c2r - cim * c2i).astype(jnp.bfloat16)
            ccat[rows, pl.ds(P, P)] = (cim * nc2r - cre * c2i).astype(jnp.bfloat16)

    def scan(ro, ng):
        last = lax.broadcasted_iota(jnp.int32, (8, 128), 0) == 7
        for c in range(NC):
            ln = pl.ds(c * 128, 128)
            hr = hst[0, :, ln]
            hi = hst[1, :, ln]

            def T(idx):
                return tab[idx, :, ln]

            def B(g, k):
                r0 = ro + g * 64 + k * 8
                return (bu_s[pl.ds(r0, 8), pl.ds(c * 128, 128)],
                        bu_s[pl.ds(r0, 8), pl.ds(P + c * 128, 128)])

            for g in range(ng):
                er, ei = B(g, 0)
                for k in range(1, 8):
                    er, ei = _cmac(*B(g, k), T(T_A), T(T_A + 1), er, ei)
                hr = pltpu.roll(jnp.where(last, hr, er), 1, 0)
                hi = pltpu.roll(jnp.where(last, hi, ei), 1, 0)
                for q, sh in enumerate((1, 2, 4)):
                    hr, hi = _cmac(hr, hi, T(T_T + 2 * q), T(T_T + 2 * q + 1),
                                   pltpu.roll(hr, sh, 0), pltpu.roll(hi, sh, 0))
                for j in range(4):
                    h0r, h0i = _cmac(*B(g, 2 * j), T(T_A), T(T_A + 1), hr, hi)
                    hr, hi = _cmac(*B(g, 2 * j + 1), T(T_A), T(T_A + 1), h0r, h0i)
                    r0 = ro + g * 64 + j * 16
                    st16(h_s, r0, pl.ds(c * 128, 128), jnp.concatenate([h0r, hr], axis=0))
                    st16(h_s, r0, pl.ds(P + c * 128, 128), jnp.concatenate([h0i, hi], axis=0))
            hst[0, :, ln] = hr
            hst[1, :, ln] = hi

    def bu_part(ro, t0, t1):
        cols = pl.ds(t0 * 128, (t1 - t0) * 128)
        bu_s[pl.ds(ro, TL), cols] = _dot(ld16(xn_s, ro, TL), bcat[cols, :], NT_DIMS)

    def gu_part(ro, ci):
        r, d0, a0 = gu_geom(ci)
        gu = _dot(ld16(xn_s, ro, TL), w13[pl.ds(d0, 2 * r), :], NT_DIMS)
        hg = 0.5 * gu[:, :r]
        st16(act_s, ro, pl.ds(a0, r), (hg * gu[:, r:]) * (1.0 + jnp.tanh(hg)))

    def down_main(ro):
        rows = pl.ds(ro, TL)
        yp_s[rows, :] = base_s[rows, :] + _dot(ld16(act_s, ro, TL, pl.ds(0, FM)),
                                               w2v[pl.ds(0, FM), :], NN_DIMS)

    def finish_col(blk, ro, c, msplit=1, gdma=False):
        cols = pl.ds(c * 128, 128)
        q = TL // msplit
        tail = [_dot(ld16(act_s, ro + k * q, q, pl.ds(FM, FT)), w2v[pl.ds(FM, FT), cols], NN_DIMS)
                for k in range(msplit)]
        yc = yp_s[pl.ds(ro, TL), cols] + jnp.concatenate(tail, axis=0)
        yc = yc + _dot(ld16(h_s, ro, TL), ccat[cols, :], NT_DIMS)
        for g in range(G):
            for k in range(8):
                r0 = g * 64 + k * 8
                obuf[blk, c, pl.ds(g * 64 + k, 8, stride=8), :] = yc[r0:r0 + 8, :]
            if gdma:
                o_copy(blk, c, g, 1).start()
        if not gdma:
            o_copy(blk, c).start()

    start(x_copies(0) + p_copies((3,)))
    start(x_copies(1))
    start(b_copies(0))
    start(p_copies((0, 1, 2)))
    for k in range(1, NBS - 1):
        start(b_copies(k))
    for k in range(NWG):
        start(group_copies(k))
    for blk in range(3, NS):
        start(x_copies(blk))
    hst[...] = jnp.zeros(hst.shape, jnp.float32)
    wait(x_copies(0) + p_copies((3,)))
    tab[T_DSK] = row8(pv[3])
    layernorm(0, 0)
    wait(x_copies(1))
    layernorm(1, TL)
    for k in range(NBS):
        wait(b_copies(k) if k < NBS - 1 else group_copies(0))
        if k == 1:
            wait(p_copies((0, 1, 2)))
            build_tables()
        bu_part(0, BB[k], BB[k + 1])
        bu_part(TL, BB[k], BB[k + 1])
    scan(0, 2 * G)
    for ci in range(NGU + 1):
        if ci > 0 and ci in WB:
            wait(group_copies(WB.index(ci)))
        gu_part(0, ci)
        gu_part(TL, ci)
    down_main(0)
    down_main(TL)
    fold_c()
    for c in range(NC):
        finish_col(0, 0, c, msplit=4 if c < 3 else 1)
    ln_stats(2)
    for blk in range(3, NS):
        wait(x_copies(blk))

    def body(i, carry):
        ln_apply(i, TL)
        for c in range(NC):
            finish_col(i - 1, TL, c)
        for c in range(NC):
            bu_part(TL, c, c + 1)
            bu_part(TL, NC + c, NC + c + 1)
        scan(TL, G)
        for ci in range(NGU + 1):
            gu_part(TL, ci)
        down_main(TL)
        ln_stats(jnp.minimum(i + 1, NS - 1))
        return carry

    lax.fori_loop(2, NS, body, 0)

    for c in range(NC):
        finish_col(NS - 1, TL, c, gdma=(c == NC - 1))
    for blk in range(NS):
        for c in range(NC):
            if (blk, c) == (NS - 1, NC - 1):
                for g in range(G):
                    o_copy(blk, c, g, 1).wait()
            else:
                o_copy(blk, c).wait()


_SCRATCH = [
    pltpu.VMEM((NS, NC, TL, 128), jnp.bfloat16),
    pltpu.VMEM((P,), jnp.bfloat16),
    pltpu.VMEM((P,), jnp.bfloat16),
    pltpu.VMEM((P,), jnp.bfloat16),
    pltpu.VMEM((D,), jnp.bfloat16),
    pltpu.VMEM((2 * P, D), jnp.bfloat16),
    pltpu.VMEM((2 * F, D), jnp.bfloat16),
    pltpu.VMEM((D, 2 * P), jnp.bfloat16),
    pltpu.VMEM((F, D), jnp.bfloat16),
    pltpu.VMEM((N_TAB, 8, P), jnp.float32),
    pltpu.VMEM((2, 8, P), jnp.float32),
    pltpu.VMEM((TL, D), jnp.uint32),
    pltpu.VMEM((2 * TL, D), jnp.float32),
    pltpu.VMEM((2 * TL, D), jnp.float32),
    pltpu.VMEM((TL, 2 * P), jnp.uint32),
    pltpu.VMEM((TL, F), jnp.uint32),
    pltpu.VMEM((NS, NC, TL, 128), jnp.float32),
    pltpu.VMEM((2 * TL, 2 * P), jnp.float32),
    pltpu.VMEM((2, TL, 128), jnp.float32),
    pltpu.SemaphoreType.DMA((N_SEM,)),
    pltpu.SemaphoreType.DMA((1,)),
]

_PARAM_NAMES = {f.name for f in dataclasses.fields(pltpu.CompilerParams)}
_PARAMS = dict(vmem_limit_bytes=100 * 1024 * 1024)
_PARAMS.update({k: True for k in ("disable_bounds_checks", "disable_semaphore_checks")
                if k in _PARAM_NAMES})


@jax.jit
def pallas_parallel_sum__ssm_conv_s5__glu_gated_swiglu__prompt_kernel(
    A_x: jax.Array,
    A_Lambda_re: jax.Array,
    A_Lambda_im: jax.Array,
    A_B_re: jax.Array,
    A_B_im: jax.Array,
    A_C_re: jax.Array,
    A_C_im: jax.Array,
    A_log_dt: jax.Array,
    A_Dskip: jax.Array,
    B_x: jax.Array,
    B_w1: jax.Array,
    B_w3: jax.Array,
    B_w2: jax.Array,
):
    del B_x
    hbm = pl.BlockSpec(memory_space=pltpu.MemorySpace.HBM)
    return pl.pallas_call(
        _kernel,
        in_specs=[hbm] * 12,
        out_specs=hbm,
        out_shape=jax.ShapeDtypeStruct((1, L, D), jnp.float32),
        scratch_shapes=_SCRATCH,
        compiler_params=pltpu.CompilerParams(**_PARAMS),
    )(A_x, A_Lambda_re, A_Lambda_im, A_B_re, A_B_im, A_C_re, A_C_im, A_log_dt, A_Dskip,
      B_w1.T, B_w3.T, B_w2)
```
